```python
import os as _os
_os.environ.setdefault("JAX_PLATFORMS", "cpu")
import jax
import jax.numpy as jnp

def _softmax(x, axis=-1):
    return jax.nn.softmax(x, axis=axis)
def _gelu(x):
    return jax.nn.gelu(x, approximate=True)
def _silu(x):
    return jax.nn.silu(x)
def _sigmoid(x):
    return jax.nn.sigmoid(x)
def _layernorm(x, axis=-1, eps=1e-5):
    m = jnp.mean(x, axis=axis, keepdims=True)
    v = jnp.var(x, axis=axis, keepdims=True)
    return (x - m) / jnp.sqrt(v + eps)
def _scatter_add(tgt, idx, src, axis=0):
    return tgt.at[idx].add(src)
def _segment_sum(src, seg, n):
    return jax.ops.segment_sum(src, seg, n)
class _Rng:
    def __init__(self, key):
        self._k = key
    def _next(self):
        self._k, sub = jax.random.split(self._k)
        return sub
    def normal(self, shape):
        return jax.random.normal(self._next(), shape, dtype=jnp.bfloat16)
    def randint(self, lo, hi, shape):
        return jax.random.randint(self._next(), shape, lo, hi, dtype=jnp.int32)
    def uniform(self, shape, lo=0.0, hi=1.0):
        return jax.random.uniform(self._next(), shape, jnp.bfloat16, lo, hi)
    def permutation(self, n):
        return jax.random.permutation(self._next(), n)


kernel_name = 'concat_heads__mha_block_cached__mha_block_cached__near_ridge'

def setup_inputs():
    _rng = _Rng(jax.random.key(int.from_bytes(__import__("os").urandom(4), "little")))
    _w = (lambda a: (lambda t: t.astype(jnp.bfloat16) if jnp.issubdtype(t.dtype, jnp.floating) else t)(jnp.asarray(a)))
    def _A_setup():
        B, Sq, D = 8, 144, 640
        H, Sk, Dh = 32, 512, 128
        return {
            "x": _w((lambda *s: _rng.normal(s) * 0.8)(B, Sq, D)),
            "k_cache": _w((lambda *s: _rng.normal(s) * 0.8)(B, H, Sk, Dh)),
            "v_cache": _w((lambda *s: _rng.normal(s) * 0.05)(B, H, Sk, Dh)),
            "wq": _w((lambda *s: _rng.normal(s) * 0.8)(D, H * Dh) * (D ** -0.5)),
            "wo": _w((lambda *s: _rng.normal(s) * 0.05)(H * Dh, D) * ((H * Dh) ** -0.5)),
        }
    _A_in = _A_setup()

    def _B_setup():
        B, Sq, D = 8, 144, 640
        H, Sk, Dh = 32, 512, 128
        return {
            "x": _w((lambda *s: _rng.normal(s) * 0.8)(B, Sq, D)),
            "k_cache": _w((lambda *s: _rng.normal(s) * 0.8)(B, H, Sk, Dh)),
            "v_cache": _w((lambda *s: _rng.normal(s) * 0.05)(B, H, Sk, Dh)),
            "wq": _w((lambda *s: _rng.normal(s) * 0.8)(D, H * Dh) * (D ** -0.5)),
            "wo": _w((lambda *s: _rng.normal(s) * 0.05)(H * Dh, D) * ((H * Dh) ** -0.5)),
        }
    _B_in = _B_setup()

    return {
        "A_x": _A_in["x"],
        "A_k_cache": _A_in["k_cache"],
        "A_v_cache": _A_in["v_cache"],
        "A_wq": _A_in["wq"],
        "A_wo": _A_in["wo"],
        "B_x": _B_in["x"],
        "B_k_cache": _B_in["k_cache"],
        "B_v_cache": _B_in["v_cache"],
        "B_wq": _B_in["wq"],
        "B_wo": _B_in["wo"],
    }

def reference(A_x, A_k_cache, A_v_cache, A_wq, A_wo, B_x, B_k_cache, B_v_cache, B_wq, B_wo):
    def _A_ref(x, k_cache, v_cache, wq, wo):
        B, Sq, D = x.shape
        H, Dh = 32, 128
        q = (lambda x, *d: x.transpose(*d))((x @ wq).reshape(B, Sq, H, Dh), 0, 2, 1, 3)
        scores = jnp.einsum("bhqd,bhkd->bhqk", q, k_cache) * (Dh ** -0.5)
        p = _softmax(scores, axis=-1)
        o = jnp.einsum("bhqk,bhkd->bhqd", p, v_cache)
        return (lambda x, *d: x.transpose(*d))(o, 0, 2, 1, 3).reshape(B, Sq, H * Dh) @ wo

    def _B_ref(x, k_cache, v_cache, wq, wo):
        B, Sq, D = x.shape
        H, Dh = 32, 128
        q = (lambda x, *d: x.transpose(*d))((x @ wq).reshape(B, Sq, H, Dh), 0, 2, 1, 3)
        scores = jnp.einsum("bhqd,bhkd->bhqk", q, k_cache) * (Dh ** -0.5)
        p = _softmax(scores, axis=-1)
        o = jnp.einsum("bhqk,bhkd->bhqd", p, v_cache)
        return (lambda x, *d: x.transpose(*d))(o, 0, 2, 1, 3).reshape(B, Sq, H * Dh) @ wo

    a = _A_ref(A_x, A_k_cache, A_v_cache, A_wq, A_wo)
    b = _B_ref(B_x, B_k_cache, B_v_cache, B_wq, B_wo)
    return jnp.concatenate([a, b], axis=-1)
```

```python
import jax
import jax.numpy as jnp
import numpy as np
from jax import lax
from jax.experimental import pallas as pl
from jax.experimental.pallas import tpu as pltpu

B, SQ, D = 8, 144, 640
H, SK, DH = 32, 512, 128
M = B * SQ
NI = 2 * H

NSL = 4
LA = 7
NQ = LA + 1
U = 7
NA = NI - 1 - LA
NTA = NA // U
UB = 3
NTB = (LA - 1) // UB
NAC = 4
KA = NTA - NAC
AC = M // NAC
G0 = 4
GB0 = B // G0
XB_ITEM = 12

assert NA == U * NTA and (LA - 1) == UB * NTB and NQ & (NQ - 1) == 0 and NSL == 4
assert U * (KA + 1) >= H + 1
assert AC % 16 == 0 and XB_ITEM < H - LA - 1

QSCALE = float((DH ** -0.5) * np.log2(np.e))
F32 = jnp.float32
BF16 = jnp.bfloat16

ORDER_MAIN = (("q", 0), ("p", 0), ("s", 0), ("o", 0), ("v", 0))
ORDER_FIRST = (("p", GB0), ("q", 0), ("s", 0), ("v", -1))
ORDER_TAIL = (("o", 0), ("q", 0), ("s", 0), ("v", -1))
ORDER_LAST = (("q", 0), ("s", 0), ("v", -1), ("x", -2), ("o", -1))


def _mha_kernel(ax, ak, av, awq, awo, bx, bk, bv, bwq, bwo, out,
                x_buf, k_buf, v_buf, wq_buf, wo_buf, q_scr, o_scr, acc, ostage,
                x_sem, k_sem, v_sem, wq_sem, wo_sem, ob_sem, first_sem, oa_sem):

    def off(idx, n):
        return idx * n if isinstance(idx, int) else pl.multiple_of(idx * n, n)

    def rows(b):
        return pl.ds(b * SQ, SQ)

    def k_copy(br, h, s):
        return pltpu.make_async_copy((ak, bk)[br].at[:, h], k_buf.at[s], k_sem.at[s])

    def v_copy(br, h, s):
        return pltpu.make_async_copy((av, bv)[br].at[:, h], v_buf.at[s], v_sem.at[s])

    def wq_copy(br, h, s):
        return pltpu.make_async_copy((awq, bwq)[br].at[:, pl.ds(off(h, DH), DH)], wq_buf.at[s], wq_sem.at[s])

    def wo_copy(br, h, s):
        return pltpu.make_async_copy((awo, bwo)[br].at[pl.ds(off(h, DH), DH), :], wo_buf.at[s], wo_sem.at[s])

    def xb_copy():
        return pltpu.make_async_copy(bx, x_buf.at[1], x_sem.at[0])

    def outa_copy(c):
        r = pl.ds(off(c, AC), AC)
        return pltpu.make_async_copy(ostage.at[0, r], out.at[r, pl.ds(0, D)], oa_sem.at[c])

    def outb_copy(b):
        return pltpu.make_async_copy(ostage.at[1, rows(b)], out.at[rows(b), pl.ds(D, D)], ob_sem.at[b])

    def start_item(j, make_copy, s):
        if isinstance(j, int):
            if j < NI:
                make_copy(j // H, j % H, s).start()
            return

        @pl.when(j < H)
        def _():
            make_copy(0, j, s).start()

        @pl.when(jnp.logical_and(j >= H, j < NI))
        def _():
            make_copy(1, j - H, s).start()

    def start_set(j, s, with_wq=True):
        if with_wq:
            start_item(j + LA, wq_copy, s)
        start_item(j, k_copy, s)
        start_item(j - 1, wo_copy, s)
        start_item(j, v_copy, s)

    S0 = NSL - 1

    def x0_copy(g):
        r = pl.ds(off(g, GB0 * SQ), GB0 * SQ)
        return pltpu.make_async_copy(ax.at[r], x_buf.at[0, r], first_sem.at[0, g])

    def k0_copy(g):
        r = pl.ds(off(g, GB0), GB0)
        return pltpu.make_async_copy(ak.at[r, 0], k_buf.at[S0, r], first_sem.at[1, g])

    def v0_copy(g):
        r = pl.ds(off(g, GB0), GB0)
        return pltpu.make_async_copy(av.at[r, 0], v_buf.at[S0, r], first_sem.at[2, g])

    def wq0_slot(j):
        return NSL + j if j < LA else S0

    wq_copy(0, 0, wq0_slot(0)).start()
    x0_copy(0).start()

    def first_wq(j, c):
        @pl.when(j < LA)
        def _():
            wq_copy(0, j, NSL + j).start()

        @pl.when(j == LA)
        def _():
            wq_copy(0, j, S0).start()
        return c
    lax.fori_loop(1, LA + 1, first_wq, 0)

    def first_kv(g, c):
        @pl.when(g + 1 < G0)
        def _():
            x0_copy(g + 1).start()
        k0_copy(g).start()
        v0_copy(g).start()
        return c
    lax.fori_loop(0, G0, first_kv, 0)

    def first_sets(j, c):
        start_set(j, j - 1)
        return c
    lax.fori_loop(1, NSL, first_sets, 0)

    def zero_acc(j, c):
        acc[j // B, pl.ds(pl.multiple_of((j % B) * SQ, 8), SQ), :] = jnp.zeros((SQ, D), F32)
        return c
    lax.fori_loop(0, 2 * B, zero_acc, 0)

    def q_projection(br, sw, sq, b):
        q = jnp.dot(x_buf[br, rows(b), :], wq_buf[sw], preferred_element_type=F32)
        q_scr[sq, rows(b), :] = (q * QSCALE).astype(BF16)

    def run_item(order, qc, oc, s, wait_k, wait_v, stage_p=None, stage_o=None, stage_x=None):
        live = {}

        def stage_q(b):
            wait_k(b)
            live["s", b] = lax.dot_general(q_scr[qc, rows(b), :], k_buf[s, b], (((1,), (1,)), ((), ())),
                                           preferred_element_type=F32)

        def stage_s(b):
            sc = live.pop(("s", b))
            m = jnp.max(sc, axis=-1, keepdims=True)
            p = jnp.exp2(sc - m)
            live["l", b] = jnp.sum(p, axis=-1, keepdims=True)
            live["p", b] = p.astype(BF16)

        def stage_v(b):
            wait_v(b)
            o = jnp.dot(live.pop(("p", b)), v_buf[s, b], preferred_element_type=F32)
            l = live.pop(("l", b))
            r = pl.reciprocal(l, approx=True)
            r = r * (2.0 - l * r)
            o_scr[oc, rows(b), :] = (o * r).astype(BF16)

        stages = dict(q=stage_q, s=stage_s, v=stage_v, p=stage_p, o=stage_o, x=stage_x)
        lo = min(o for _, o in order)
        hi = max(o for _, o in order)
        for t in range(-hi, B - lo):
            for name, o in order:
                if 0 <= t + o < B and stages[name] is not None:
                    stages[name](t + o)

    def at_first_block(fn):
        def wait(b):
            if b == 0:
                fn()
        return wait

    def make_stage_p(br, s, qn):
        def stage_p(b):
            if b == 0:
                wq_copy(0, 0, s).wait()
            q_projection(br, s, qn, b)
        return stage_p

    def make_stage_o(br, s, oc):
        def stage_o(b):
            if b == 0:
                wo_copy(0, 0, s).wait()
            acc[br, rows(b), :] += jnp.dot(o_scr[1 - oc, rows(b), :], wo_buf[s], preferred_element_type=F32)
        return stage_o

    def wait_k_of(s):
        return at_first_block(lambda: k_copy(0, 0, s).wait())

    def wait_v_of(s):
        return at_first_block(lambda: v_copy(0, 0, s).wait())

    def first_p(b):
        if b % GB0 == 0:
            x0_copy(b // GB0).wait()
        if b == 0:
            for j in range(LA + 1):
                wq_copy(0, j, wq0_slot(j)).wait()
                for bb in range(GB0):
                    q_projection(0, wq0_slot(j), j, bb)
        elif b >= GB0:
            for j in range(LA + 1):
                q_projection(0, wq0_slot(j), j, b)

    def first_wait_k(b):
        if b % GB0 == 0:
            k0_copy(b // GB0).wait()

    def first_wait_v(b):
        if b % GB0 == 0:
            v0_copy(b // GB0).wait()

    run_item(ORDER_FIRST, 0, 0, S0, first_wait_k, first_wait_v, stage_p=first_p)
    start_set(NSL, S0)

    def main_trip(k, carry):
        for u in range(U):
            i = 1 + U * k + u
            s = (i - 1) & (NSL - 1)
            qc = i & (NQ - 1)
            qn = (i + LA) & (NQ - 1)
            oc = i & 1
            br_next = jnp.where(i + LA >= H, 1, 0)
            br_prev = jnp.where(i - 1 >= H, 1, 0)
            run_item(ORDER_MAIN, qc, oc, s, wait_k_of(s), wait_v_of(s),
                     stage_p=make_stage_p(br_next, s, qn), stage_o=make_stage_o(br_prev, s, oc))
            start_set(i + NSL, s)
            if u == (XB_ITEM - 1) % U:
                @pl.when(i == XB_ITEM)
                def _():
                    xb_copy().start()
            if u == (H - LA - 2) % U:
                @pl.when(i == H - LA - 1)
                def _():
                    xb_copy().wait()
        c = jnp.maximum(k - KA, 0)
        r = pl.ds(off(c, AC), AC)
        ostage[0, r, :] = acc[0, r, :].astype(BF16)

        @pl.when(k >= KA)
        def _():
            outa_copy(c).start()
        return carry

    lax.fori_loop(0, NTA, main_trip, 0)

    def tail_trip(t, carry):
        for u in range(UB):
            i = NA + 1 + UB * t + u
            s = (i - 1) & (NSL - 1)
            oc = i & 1
            run_item(ORDER_TAIL, i & (NQ - 1), oc, s, wait_k_of(s), wait_v_of(s),
                     stage_o=make_stage_o(1, s, oc))
            start_set(i + NSL, s, with_wq=False)
        return carry

    lax.fori_loop(0, NTB, tail_trip, 0)

    last = NI - 1
    s_last = (last - 1) % NSL
    s_wo = last % NSL

    def final_projection(b):
        if b == 0:
            wo_copy(0, 0, s_wo).wait()
        r = acc[1, rows(b), :] + jnp.dot(o_scr[last % 2, rows(b), :], wo_buf[s_wo], preferred_element_type=F32)
        ostage[1, rows(b), :] = r.astype(BF16)
        outb_copy(b).start()

    run_item(ORDER_LAST, last % NQ, last % 2, s_last, wait_k_of(s_last), wait_v_of(s_last),
             stage_o=make_stage_o(1, s_last, last % 2), stage_x=final_projection)

    for c in range(NAC):
        outa_copy(c).wait()
    for b in range(B):
        outb_copy(b).wait()


@jax.jit
def pallas_concat_heads__mha_block_cached__mha_block_cached__near_ridge_kernel(
    A_x: jax.Array,
    A_k_cache: jax.Array,
    A_v_cache: jax.Array,
    A_wq: jax.Array,
    A_wo: jax.Array,
    B_x: jax.Array,
    B_k_cache: jax.Array,
    B_v_cache: jax.Array,
    B_wq: jax.Array,
    B_wo: jax.Array,
):
    assert A_x.shape == (B, SQ, D) and A_k_cache.shape == (B, H, SK, DH)
    hbm = pl.BlockSpec(memory_space=pl.ANY)
    out = pl.pallas_call(
        _mha_kernel,
        in_specs=[hbm] * 10,
        out_specs=hbm,
        out_shape=jax.ShapeDtypeStruct((M, 2 * D), BF16),
        scratch_shapes=[
            pltpu.VMEM((2, M, D), BF16),
            pltpu.VMEM((NSL, B, SK, DH), BF16),
            pltpu.VMEM((NSL, B, SK, DH), BF16),
            pltpu.VMEM((NSL + LA, D, DH), BF16),
            pltpu.VMEM((NSL, DH, D), BF16),
            pltpu.VMEM((NQ, M, DH), BF16),
            pltpu.VMEM((2, M, DH), BF16),
            pltpu.VMEM((2, M, D), F32),
            pltpu.VMEM((2, M, D), BF16),
            pltpu.SemaphoreType.DMA((1,)),
            pltpu.SemaphoreType.DMA((NSL,)),
            pltpu.SemaphoreType.DMA((NSL,)),
            pltpu.SemaphoreType.DMA((NSL + LA,)),
            pltpu.SemaphoreType.DMA((NSL,)),
            pltpu.SemaphoreType.DMA((B,)),
            pltpu.SemaphoreType.DMA((3, G0)),
            pltpu.SemaphoreType.DMA((NAC,)),
        ],
        compiler_params=pltpu.CompilerParams(
            vmem_limit_bytes=100 * 1024 * 1024,
            disable_bounds_checks=True,
            disable_semaphore_checks=True,
            flags={"XLA_TPU_RESCHEDULE_DMA_DONES": True},
        ),
    )(A_x.reshape(M, D), A_k_cache, A_v_cache, A_wq, A_wo,
      B_x.reshape(M, D), B_k_cache, B_v_cache, B_wq, B_wo)
    return out.reshape(B, SQ, 2 * D)
```

```python
import jax
import jax.numpy as jnp
import numpy as np
from jax import lax
from jax.experimental import pallas as pl
from jax.experimental.pallas import tpu as pltpu

B, SQ, D = 8, 144, 640
H, SK, DH = 32, 512, 128
M = B * SQ
NI = 2 * H

NSL = 4
LA = 7
NQ = LA + 1
U = 7
NA = NI - 1 - LA
NTA = NA // U
UB = 3
NTB = (LA - 1) // UB
NAC = 4
KA = NTA - NAC
AC = M // NAC
G0 = 4
GB0 = B // G0
XB_ITEM = 12

assert NA == U * NTA and (LA - 1) == UB * NTB and NQ & (NQ - 1) == 0 and NSL == 4
assert U * (KA + 1) >= H + 1
assert AC % 16 == 0 and XB_ITEM < H - LA - 1

QSCALE = float((DH ** -0.5) * np.log2(np.e))
F32 = jnp.float32
BF16 = jnp.bfloat16

ORDER_MAIN = (("q", 0), ("p", 0), ("s", 0), ("o", 0), ("v", 0))
ORDER_FIRST = (("p", GB0), ("q", 0), ("s", 0), ("v", -1))
ORDER_TAIL = (("o", 0), ("q", 0), ("s", 0), ("v", -1))
ORDER_LAST = (("q", 0), ("s", 0), ("v", -1), ("x", -2), ("o", -1))


def _mha_kernel(ax, ak, av, awq, awo, bx, bk, bv, bwq, bwo, out,
                x_buf, k_buf, v_buf, wq_buf, wo_buf, q_scr, o_scr, acc, ostage,
                x_sem, k_sem, v_sem, wq_sem, wo_sem, ob_sem, first_sem, oa_sem):

    def off(idx, n):
        return idx * n if isinstance(idx, int) else pl.multiple_of(idx * n, n)

    def rows(b):
        return pl.ds(b * SQ, SQ)

    def k_copy(br, h, s):
        return pltpu.make_async_copy((ak, bk)[br].at[:, h], k_buf.at[s], k_sem.at[s])

    def v_copy(br, h, s):
        return pltpu.make_async_copy((av, bv)[br].at[:, h], v_buf.at[s], v_sem.at[s])

    def wq_copy(br, h, s):
        return pltpu.make_async_copy((awq, bwq)[br].at[:, pl.ds(off(h, DH), DH)], wq_buf.at[s], wq_sem.at[s])

    def wo_copy(br, h, s):
        return pltpu.make_async_copy((awo, bwo)[br].at[pl.ds(off(h, DH), DH), :], wo_buf.at[s], wo_sem.at[s])

    def xb_copy():
        return pltpu.make_async_copy(bx, x_buf.at[1], x_sem.at[0])

    def outa_copy(c):
        r = pl.ds(off(c, AC), AC)
        return pltpu.make_async_copy(ostage.at[0, r], out.at[r, pl.ds(0, D)], oa_sem.at[c])

    def outb_copy(b):
        return pltpu.make_async_copy(ostage.at[1, rows(b)], out.at[rows(b), pl.ds(D, D)], ob_sem.at[b])

    def start_item(j, make_copy, s):
        if isinstance(j, int):
            if j < NI:
                make_copy(j // H, j % H, s).start()
            return

        @pl.when(j < H)
        def _():
            make_copy(0, j, s).start()

        @pl.when(jnp.logical_and(j >= H, j < NI))
        def _():
            make_copy(1, j - H, s).start()

    def start_set(j, s, with_wq=True):
        if with_wq:
            start_item(j + LA, wq_copy, s)
        start_item(j, k_copy, s)
        start_item(j - 1, wo_copy, s)
        start_item(j, v_copy, s)

    S0 = NSL - 1

    def x0_copy(g):
        r = pl.ds(off(g, GB0 * SQ), GB0 * SQ)
        return pltpu.make_async_copy(ax.at[r], x_buf.at[0, r], first_sem.at[0, g])

    def k0_copy(g):
        r = pl.ds(off(g, GB0), GB0)
        return pltpu.make_async_copy(ak.at[r, 0], k_buf.at[S0, r], first_sem.at[1, g])

    def v0_copy(g):
        r = pl.ds(off(g, GB0), GB0)
        return pltpu.make_async_copy(av.at[r, 0], v_buf.at[S0, r], first_sem.at[2, g])

    def wq0_slot(j):
        return NSL + j if j < LA else S0

    wq_copy(0, 0, wq0_slot(0)).start()
    x0_copy(0).start()

    def first_wq(j, c):
        @pl.when(j < LA)
        def _():
            wq_copy(0, j, NSL + j).start()

        @pl.when(j == LA)
        def _():
            wq_copy(0, j, S0).start()
        return c
    lax.fori_loop(1, LA + 1, first_wq, 0)

    def first_kv(g, c):
        @pl.when(g + 1 < G0)
        def _():
            x0_copy(g + 1).start()
        k0_copy(g).start()
        v0_copy(g).start()
        return c
    lax.fori_loop(0, G0, first_kv, 0)

    def first_sets(j, c):
        start_set(j, j - 1)
        return c
    lax.fori_loop(1, NSL, first_sets, 0)

    def zero_acc(j, c):
        acc[j // B, pl.ds(pl.multiple_of((j % B) * SQ, 8), SQ), :] = jnp.zeros((SQ, D), F32)
        return c
    lax.fori_loop(0, 2 * B, zero_acc, 0)

    def q_projection(br, sw, sq, b):
        q = jnp.dot(x_buf[br, rows(b), :], wq_buf[sw], preferred_element_type=F32)
        q_scr[sq, rows(b), :] = (q * QSCALE).astype(BF16)

    def run_item(order, qc, oc, s, wait_k, wait_v, stage_p=None, stage_o=None, stage_x=None):
        live = {}

        def stage_q(b):
            wait_k(b)
            live["s", b] = lax.dot_general(q_scr[qc, rows(b), :], k_buf[s, b], (((1,), (1,)), ((), ())),
                                           preferred_element_type=F32)

        def stage_s(b):
            sc = live.pop(("s", b))
            m = jnp.max(sc, axis=-1, keepdims=True)
            p = jnp.exp2(sc - m)
            live["l", b] = jnp.sum(p, axis=-1, keepdims=True)
            live["p", b] = p.astype(BF16)

        def stage_v(b):
            wait_v(b)
            o = jnp.dot(live.pop(("p", b)), v_buf[s, b], preferred_element_type=F32)
            l = live.pop(("l", b))
            r = pl.reciprocal(l, approx=True)
            r = r * (2.0 - l * r)
            o_scr[oc, rows(b), :] = (o * r).astype(BF16)

        stages = dict(q=stage_q, s=stage_s, v=stage_v, p=stage_p, o=stage_o, x=stage_x)
        lo = min(o for _, o in order)
        hi = max(o for _, o in order)
        for t in range(-hi, B - lo):
            for name, o in order:
                if 0 <= t + o < B and stages[name] is not None:
                    stages[name](t + o)

    def at_first_block(fn):
        def wait(b):
            if b == 0:
                fn()
        return wait

    def make_stage_p(br, s, qn):
        def stage_p(b):
            if b == 0:
                wq_copy(0, 0, s).wait()
            q_projection(br, s, qn, b)
        return stage_p

    def make_stage_o(br, s, oc):
        def stage_o(b):
            if b == 0:
                wo_copy(0, 0, s).wait()
            acc[br, rows(b), :] += jnp.dot(o_scr[1 - oc, rows(b), :], wo_buf[s], preferred_element_type=F32)
        return stage_o

    def wait_k_of(s):
        return at_first_block(lambda: k_copy(0, 0, s).wait())

    def wait_v_of(s):
        return at_first_block(lambda: v_copy(0, 0, s).wait())

    def first_p(b):
        if b % GB0 == 0:
            x0_copy(b // GB0).wait()
        if b == 0:
            for j in range(LA + 1):
                wq_copy(0, j, wq0_slot(j)).wait()
                for bb in range(GB0):
                    q_projection(0, wq0_slot(j), j, bb)
        elif b >= GB0:
            for j in range(LA + 1):
                q_projection(0, wq0_slot(j), j, b)

    def first_wait_k(b):
        if b % GB0 == 0:
            k0_copy(b // GB0).wait()

    def first_wait_v(b):
        if b % GB0 == 0:
            v0_copy(b // GB0).wait()

    def first_item():
        run_item(ORDER_FIRST, 0, 0, S0, first_wait_k, first_wait_v, stage_p=first_p)
        start_set(NSL, S0)

    def main_trip(k, carry):
        for u in range(U):
            i = 1 + U * k + u
            s = (i - 1) & (NSL - 1)
            qc = i & (NQ - 1)
            qn = (i + LA) & (NQ - 1)
            oc = i & 1
            br_next = jnp.where(i + LA >= H, 1, 0)
            br_prev = jnp.where(i - 1 >= H, 1, 0)
            run_item(ORDER_MAIN, qc, oc, s, wait_k_of(s), wait_v_of(s),
                     stage_p=make_stage_p(br_next, s, qn), stage_o=make_stage_o(br_prev, s, oc))
            start_set(i + NSL, s)
            if u == (XB_ITEM - 1) % U:
                @pl.when(i == XB_ITEM)
                def _():
                    xb_copy().start()
            if u == (H - LA - 2) % U:
                @pl.when(i == H - LA - 1)
                def _():
                    xb_copy().wait()
        c = jnp.maximum(k - KA, 0)
        r = pl.ds(off(c, AC), AC)
        ostage[0, r, :] = acc[0, r, :].astype(BF16)

        @pl.when(k >= KA)
        def _():
            outa_copy(c).start()
        return carry

    def tail_trip(t, carry):
        for u in range(UB):
            i = NA + 1 + UB * t + u
            s = (i - 1) & (NSL - 1)
            oc = i & 1
            run_item(ORDER_TAIL, i & (NQ - 1), oc, s, wait_k_of(s), wait_v_of(s),
                     stage_o=make_stage_o(1, s, oc))
            start_set(i + NSL, s, with_wq=False)
        return carry

    last = NI - 1
    s_last = (last - 1) % NSL
    s_wo = last % NSL

    def final_projection(b):
        if b == 0:
            wo_copy(0, 0, s_wo).wait()
        r = acc[1, rows(b), :] + jnp.dot(o_scr[last % 2, rows(b), :], wo_buf[s_wo], preferred_element_type=F32)
        ostage[1, rows(b), :] = r.astype(BF16)
        outb_copy(b).start()

    def last_item():
        run_item(ORDER_LAST, last % NQ, last % 2, s_last, wait_k_of(s_last), wait_v_of(s_last),
                 stage_o=make_stage_o(1, s_last, last % 2), stage_x=final_projection)

    def all_phases(n, carry):
        @pl.when(n == 0)
        def _():
            first_item()
            lax.fori_loop(0, NTA, main_trip, 0)
            lax.fori_loop(0, NTB, tail_trip, 0)
            last_item()
        return carry

    lax.fori_loop(0, 2, all_phases, 0)

    for c in range(NAC):
        outa_copy(c).wait()
    for b in range(B):
        outb_copy(b).wait()


@jax.jit
def pallas_concat_heads__mha_block_cached__mha_block_cached__near_ridge_kernel(
    A_x: jax.Array,
    A_k_cache: jax.Array,
    A_v_cache: jax.Array,
    A_wq: jax.Array,
    A_wo: jax.Array,
    B_x: jax.Array,
    B_k_cache: jax.Array,
    B_v_cache: jax.Array,
    B_wq: jax.Array,
    B_wo: jax.Array,
):
    assert A_x.shape == (B, SQ, D) and A_k_cache.shape == (B, H, SK, DH)
    hbm = pl.BlockSpec(memory_space=pl.ANY)
    out = pl.pallas_call(
        _mha_kernel,
        in_specs=[hbm] * 10,
        out_specs=hbm,
        out_shape=jax.ShapeDtypeStruct((M, 2 * D), BF16),
        scratch_shapes=[
            pltpu.VMEM((2, M, D), BF16),
            pltpu.VMEM((NSL, B, SK, DH), BF16),
            pltpu.VMEM((NSL, B, SK, DH), BF16),
            pltpu.VMEM((NSL + LA, D, DH), BF16),
            pltpu.VMEM((NSL, DH, D), BF16),
            pltpu.VMEM((NQ, M, DH), BF16),
            pltpu.VMEM((2, M, DH), BF16),
            pltpu.VMEM((2, M, D), F32),
            pltpu.VMEM((2, M, D), BF16),
            pltpu.SemaphoreType.DMA((1,)),
            pltpu.SemaphoreType.DMA((NSL,)),
            pltpu.SemaphoreType.DMA((NSL,)),
            pltpu.SemaphoreType.DMA((NSL + LA,)),
            pltpu.SemaphoreType.DMA((NSL,)),
            pltpu.SemaphoreType.DMA((B,)),
            pltpu.SemaphoreType.DMA((3, G0)),
            pltpu.SemaphoreType.DMA((NAC,)),
        ],
        compiler_params=pltpu.CompilerParams(
            vmem_limit_bytes=100 * 1024 * 1024,
            disable_bounds_checks=True,
            disable_semaphore_checks=True,
            flags={"XLA_TPU_RESCHEDULE_DMA_DONES": True},
        ),
    )(A_x.reshape(M, D), A_k_cache, A_v_cache, A_wq, A_wo,
      B_x.reshape(M, D), B_k_cache, B_v_cache, B_wq, B_wo)
    return out.reshape(B, SQ, 2 * D)
```

```python
import jax
import jax.numpy as jnp
import numpy as np
from jax import lax
from jax.experimental import pallas as pl
from jax.experimental.pallas import tpu as pltpu

B, SQ, D = 8, 144, 640
H, SK, DH = 32, 512, 128
M = B * SQ
NI = 2 * H

NSL = 4
LA = 7
NQ = LA + 1
U = 7
NA = NI - 1 - LA
NTA = NA // U
UB = 3
NTB = (LA - 1) // UB
NAC = 4
KA = NTA - NAC
AC = M // NAC
G0 = 4
GB0 = B // G0
XB_ITEM = 12

assert NA == U * NTA and (LA - 1) == UB * NTB and NQ & (NQ - 1) == 0 and NSL == 4
assert U * (KA + 1) >= H + 1
assert AC % 16 == 0 and XB_ITEM < H - LA - 1

QSCALE = float((DH ** -0.5) * np.log2(np.e))
F32 = jnp.float32
BF16 = jnp.bfloat16

ORDER_MAIN = (("q", 0), ("p", 0), ("s", 0), ("o", 0), ("v", 0))
ORDER_FIRST = (("p", GB0), ("q", 0), ("s", 0), ("v", -1))
ORDER_TAIL = (("o", 0), ("q", 0), ("s", 0), ("v", -1))
ORDER_LAST = (("q", 0), ("s", 0), ("v", -1), ("x", -2), ("o", -1))


def _mha_kernel(ax, ak, av, awq, awo, bx, bk, bv, bwq, bwo, out,
                x_buf, k_buf, v_buf, wq_buf, wo_buf, q_scr, o_scr, s_scr, acc, ostage,
                x_sem, k_sem, v_sem, wq_sem, wo_sem, ob_sem, first_sem, oa_sem):

    def off(idx, n):
        return idx * n if isinstance(idx, int) else pl.multiple_of(idx * n, n)

    def rows(b):
        return pl.ds(b * SQ, SQ)

    def k_copy(br, h, s):
        return pltpu.make_async_copy((ak, bk)[br].at[:, h], k_buf.at[s], k_sem.at[s])

    def v_copy(br, h, s):
        return pltpu.make_async_copy((av, bv)[br].at[:, h], v_buf.at[s], v_sem.at[s])

    def wq_copy(br, h, s):
        return pltpu.make_async_copy((awq, bwq)[br].at[:, pl.ds(off(h, DH), DH)], wq_buf.at[s], wq_sem.at[s])

    def wo_copy(br, h, s):
        return pltpu.make_async_copy((awo, bwo)[br].at[pl.ds(off(h, DH), DH), :], wo_buf.at[s], wo_sem.at[s])

    def xb_copy():
        return pltpu.make_async_copy(bx, x_buf.at[1], x_sem.at[0])

    def outa_copy(c):
        r = pl.ds(off(c, AC), AC)
        return pltpu.make_async_copy(ostage.at[0, r], out.at[r, pl.ds(0, D)], oa_sem.at[c])

    def outb_copy(b):
        return pltpu.make_async_copy(ostage.at[1, rows(b)], out.at[rows(b), pl.ds(D, D)], ob_sem.at[b])

    def start_item(j, make_copy, s):
        if isinstance(j, int):
            if j < NI:
                make_copy(j // H, j % H, s).start()
            return

        @pl.when(j < H)
        def _():
            make_copy(0, j, s).start()

        @pl.when(jnp.logical_and(j >= H, j < NI))
        def _():
            make_copy(1, j - H, s).start()

    def start_set(j, s, with_wq=True):
        if with_wq:
            start_item(j + LA, wq_copy, s)
        start_item(j, k_copy, s)
        start_item(j - 1, wo_copy, s)
        start_item(j, v_copy, s)

    S0 = NSL - 1

    def x0_copy(g):
        r = pl.ds(off(g, GB0 * SQ), GB0 * SQ)
        return pltpu.make_async_copy(ax.at[r], x_buf.at[0, r], first_sem.at[0, g])

    def k0_copy(g):
        r = pl.ds(off(g, GB0), GB0)
        return pltpu.make_async_copy(ak.at[r, 0], k_buf.at[S0, r], first_sem.at[1, g])

    def v0_copy(g):
        r = pl.ds(off(g, GB0), GB0)
        return pltpu.make_async_copy(av.at[r, 0], v_buf.at[S0, r], first_sem.at[2, g])

    def wq0_slot(j):
        return NSL + j if j < LA else S0

    wq_copy(0, 0, wq0_slot(0)).start()
    x0_copy(0).start()

    def first_wq(j, c):
        @pl.when(j < LA)
        def _():
            wq_copy(0, j, NSL + j).start()

        @pl.when(j == LA)
        def _():
            wq_copy(0, j, S0).start()
        return c
    lax.fori_loop(1, LA + 1, first_wq, 0)

    def first_kv(g, c):
        @pl.when(g + 1 < G0)
        def _():
            x0_copy(g + 1).start()
        k0_copy(g).start()
        v0_copy(g).start()
        return c
    lax.fori_loop(0, G0, first_kv, 0)

    def first_sets(j, c):
        start_set(j, j - 1)
        return c
    lax.fori_loop(1, NSL, first_sets, 0)

    def zero_acc(j, c):
        acc[j // B, pl.ds(pl.multiple_of((j % B) * SQ, 8), SQ), :] = jnp.zeros((SQ, D), F32)
        return c
    lax.fori_loop(0, 2 * B, zero_acc, 0)

    def q_projection(br, sw, sq, b):
        q = jnp.dot(x_buf[br, rows(b), :], wq_buf[sw], preferred_element_type=F32)
        q_scr[sq, rows(b), :] = (q * QSCALE).astype(BF16)

    def scores(sq, s, b):
        return lax.dot_general(q_scr[sq, rows(b), :], k_buf[s, b], (((1,), (1,)), ((), ())),
                               preferred_element_type=F32)

    def run_item(order, qc, oc, s, wait_k, wait_v, stage_p=None, stage_o=None, stage_x=None,
                 staged=False, next_item=None):
        live = {}

        def stage_q(b):
            if staged and b == 0:
                live["s", b] = s_scr[...]
            else:
                wait_k(b)
                live["s", b] = scores(qc, s, b)

        def stage_s(b):
            sc = live.pop(("s", b))
            m = jnp.max(sc, axis=-1, keepdims=True)
            p = jnp.exp2(sc - m)
            live["l", b] = jnp.sum(p, axis=-1, keepdims=True)
            live["p", b] = p.astype(BF16)

        def stage_v(b):
            wait_v(b)
            o = jnp.dot(live.pop(("p", b)), v_buf[s, b], preferred_element_type=F32)
            l = live.pop(("l", b))
            r = pl.reciprocal(l, approx=True)
            r = r * (2.0 - l * r)
            o_scr[oc, rows(b), :] = (o * r).astype(BF16)

        stages = dict(q=stage_q, s=stage_s, v=stage_v, p=stage_p, o=stage_o, x=stage_x)
        lo = min(o for _, o in order)
        hi = max(o for _, o in order)
        for t in range(-hi, B - lo):
            for name, o in order:
                if 0 <= t + o < B and stages[name] is not None:
                    stages[name](t + o)
        if next_item is not None:
            qn, sn = next_item
            k_copy(0, 0, sn).wait()
            s_scr[...] = scores(qn, sn, 0)

    def at_first_block(fn):
        def wait(b):
            if b == 0:
                fn()
        return wait

    def make_stage_p(br, s, qn):
        def stage_p(b):
            if b == 0:
                wq_copy(0, 0, s).wait()
            q_projection(br, s, qn, b)
        return stage_p

    def make_stage_o(br, s, oc):
        def stage_o(b):
            if b == 0:
                wo_copy(0, 0, s).wait()
            acc[br, rows(b), :] += jnp.dot(o_scr[1 - oc, rows(b), :], wo_buf[s], preferred_element_type=F32)
        return stage_o

    def wait_k_of(s):
        return at_first_block(lambda: k_copy(0, 0, s).wait())

    def wait_v_of(s):
        return at_first_block(lambda: v_copy(0, 0, s).wait())

    def first_p(b):
        if b % GB0 == 0:
            x0_copy(b // GB0).wait()
        if b == 0:
            for j in range(LA + 1):
                wq_copy(0, j, wq0_slot(j)).wait()
                for bb in range(GB0):
                    q_projection(0, wq0_slot(j), j, bb)
        elif b >= GB0:
            for j in range(LA + 1):
                q_projection(0, wq0_slot(j), j, b)

    def first_wait_k(b):
        if b % GB0 == 0:
            k0_copy(b // GB0).wait()

    def first_wait_v(b):
        if b % GB0 == 0:
            v0_copy(b // GB0).wait()

    def first_item():
        run_item(ORDER_FIRST, 0, 0, S0, first_wait_k, first_wait_v, stage_p=first_p, next_item=(1, 0))
        start_set(NSL, S0)

    def successor(i):
        return (i + 1) & (NQ - 1), i & (NSL - 1)

    def main_trip(k, carry):
        for u in range(U):
            i = 1 + U * k + u
            s = (i - 1) & (NSL - 1)
            qc = i & (NQ - 1)
            qn = (i + LA) & (NQ - 1)
            oc = i & 1
            br_next = jnp.where(i + LA >= H, 1, 0)
            br_prev = jnp.where(i - 1 >= H, 1, 0)
            run_item(ORDER_MAIN, qc, oc, s, wait_k_of(s), wait_v_of(s),
                     stage_p=make_stage_p(br_next, s, qn), stage_o=make_stage_o(br_prev, s, oc),
                     staged=u == 0, next_item=successor(i) if u == U - 1 else None)
            start_set(i + NSL, s)
            if u == (XB_ITEM - 1) % U:
                @pl.when(i == XB_ITEM)
                def _():
                    xb_copy().start()
            if u == (H - LA - 2) % U:
                @pl.when(i == H - LA - 1)
                def _():
                    xb_copy().wait()
        c = jnp.maximum(k - KA, 0)
        r = pl.ds(off(c, AC), AC)
        ostage[0, r, :] = acc[0, r, :].astype(BF16)

        @pl.when(k >= KA)
        def _():
            outa_copy(c).start()
        return carry

    def tail_trip(t, carry):
        for u in range(UB):
            i = NA + 1 + UB * t + u
            s = (i - 1) & (NSL - 1)
            oc = i & 1
            run_item(ORDER_TAIL, i & (NQ - 1), oc, s, wait_k_of(s), wait_v_of(s),
                     stage_o=make_stage_o(1, s, oc),
                     staged=u == 0, next_item=successor(i) if u == UB - 1 else None)
            start_set(i + NSL, s, with_wq=False)
        return carry

    last = NI - 1
    s_last = (last - 1) % NSL
    s_wo = last % NSL

    def final_projection(b):
        if b == 0:
            wo_copy(0, 0, s_wo).wait()
        r = acc[1, rows(b), :] + jnp.dot(o_scr[last % 2, rows(b), :], wo_buf[s_wo], preferred_element_type=F32)
        ostage[1, rows(b), :] = r.astype(BF16)
        outb_copy(b).start()

    def last_item():
        run_item(ORDER_LAST, last % NQ, last % 2, s_last, wait_k_of(s_last), wait_v_of(s_last),
                 stage_o=make_stage_o(1, s_last, last % 2), stage_x=final_projection, staged=True)

    def all_phases(n, carry):
        @pl.when(n == 0)
        def _():
            first_item()
            lax.fori_loop(0, NTA, main_trip, 0)
            lax.fori_loop(0, NTB, tail_trip, 0)
            last_item()
        return carry

    lax.fori_loop(0, 2, all_phases, 0)

    for c in range(NAC):
        outa_copy(c).wait()
    for b in range(B):
        outb_copy(b).wait()


@jax.jit
def pallas_concat_heads__mha_block_cached__mha_block_cached__near_ridge_kernel(
    A_x: jax.Array,
    A_k_cache: jax.Array,
    A_v_cache: jax.Array,
    A_wq: jax.Array,
    A_wo: jax.Array,
    B_x: jax.Array,
    B_k_cache: jax.Array,
    B_v_cache: jax.Array,
    B_wq: jax.Array,
    B_wo: jax.Array,
):
    assert A_x.shape == (B, SQ, D) and A_k_cache.shape == (B, H, SK, DH)
    hbm = pl.BlockSpec(memory_space=pl.ANY)
    out = pl.pallas_call(
        _mha_kernel,
        in_specs=[hbm] * 10,
        out_specs=hbm,
        out_shape=jax.ShapeDtypeStruct((M, 2 * D), BF16),
        scratch_shapes=[
            pltpu.VMEM((2, M, D), BF16),
            pltpu.VMEM((NSL, B, SK, DH), BF16),
            pltpu.VMEM((NSL, B, SK, DH), BF16),
            pltpu.VMEM((NSL + LA, D, DH), BF16),
            pltpu.VMEM((NSL, DH, D), BF16),
            pltpu.VMEM((NQ, M, DH), BF16),
            pltpu.VMEM((2, M, DH), BF16),
            pltpu.VMEM((SQ, SK), F32),
            pltpu.VMEM((2, M, D), F32),
            pltpu.VMEM((2, M, D), BF16),
            pltpu.SemaphoreType.DMA((1,)),
            pltpu.SemaphoreType.DMA((NSL,)),
            pltpu.SemaphoreType.DMA((NSL,)),
            pltpu.SemaphoreType.DMA((NSL + LA,)),
            pltpu.SemaphoreType.DMA((NSL,)),
            pltpu.SemaphoreType.DMA((B,)),
            pltpu.SemaphoreType.DMA((3, G0)),
            pltpu.SemaphoreType.DMA((NAC,)),
        ],
        compiler_params=pltpu.CompilerParams(
            vmem_limit_bytes=100 * 1024 * 1024,
            disable_bounds_checks=True,
            disable_semaphore_checks=True,
            flags={"XLA_TPU_RESCHEDULE_DMA_DONES": True},
        ),
    )(A_x.reshape(M, D), A_k_cache, A_v_cache, A_wq, A_wo,
      B_x.reshape(M, D), B_k_cache, B_v_cache, B_wq, B_wo)
    return out.reshape(B, SQ, 2 * D)
```
